```python
import jax
import jax.numpy as jnp

def _softmax(x, axis=-1):
    return jax.nn.softmax(x, axis=axis)
def _gelu(x):
    return jax.nn.gelu(x, approximate=True)
def _silu(x):
    return jax.nn.silu(x)
def _sigmoid(x):
    return jax.nn.sigmoid(x)
def _layernorm(x, axis=-1, eps=1e-5):
    m = jnp.mean(x, axis=axis, keepdims=True)
    v = jnp.var(x, axis=axis, keepdims=True)
    return (x - m) / jnp.sqrt(v + eps)
def _scatter_add(tgt, idx, src, axis=0):
    return tgt.at[idx].add(src)
def _segment_sum(src, seg, n):
    return jax.ops.segment_sum(src, seg, n)
class _Rng:
    def __init__(self, key):
        self._k = key
    def _next(self):
        self._k, sub = jax.random.split(self._k)
        return sub
    def normal(self, shape):
        return jax.random.normal(self._next(), shape, dtype=jnp.bfloat16)
    def randint(self, lo, hi, shape):
        return jax.random.randint(self._next(), shape, lo, hi, dtype=jnp.int32)
    def uniform(self, shape, lo=0.0, hi=1.0):
        return jax.random.uniform(self._next(), shape, jnp.bfloat16, lo, hi)
    def permutation(self, n):
        return jax.random.permutation(self._next(), n)


kernel_name = 'standalone__mha_softmax__near_ridge'

def _fwd_setup_inputs():
    _rng = _Rng(jax.random.key(int.from_bytes(__import__("os").urandom(4), "little")))
    _w = (lambda a: (lambda t: t.astype(jnp.bfloat16) if jnp.issubdtype(t.dtype, jnp.floating) else t)(jnp.asarray(a)))
    B, H, Sq, Sk, D = 16, 32, 384, 1024, 128
    return {
        "q": _w((lambda *s: _rng.normal(s) * 0.05)(B, H, Sq, D)),
        "k": _w((lambda *s: _rng.normal(s) * 0.05)(B, H, Sk, D)),
        "v": _w((lambda *s: _rng.normal(s) * 0.05)(B, H, Sk, D)),
    }

def _fwd_reference(q, k, v):
    scale = q.shape[-1] ** -0.5
    scores = jnp.einsum("bhqd,bhkd->bhqk", q, k) * scale
    p = _softmax(scores, axis=-1)
    return jnp.einsum("bhqk,bhkd->bhqd", p, v)


def setup_inputs():
    _inp = _fwd_setup_inputs()
    _gk = jax.random.fold_in(jax.random.key(int.from_bytes(__import__("os").urandom(4), "little")), 2**31 - 1)
    _shapes = [[16, 32, 384, 128]]
    _dtypes = ['bfloat16']
    _gks = jax.random.split(_gk, len(_shapes))
    _gs = [jax.random.normal(k, s, dtype=jnp.dtype(d)) * 0.05 for k, s, d in zip(_gks, _shapes, _dtypes)]
    _inp["grad_out"] = _gs[0]
    return _inp

def reference(q, k, v, grad_out):
    _const = dict()
    def _f(*_d):
        return _fwd_reference(**{'q': _d[0], 'k': _d[1], 'v': _d[2], **_const})
    _out, _vjp = jax.vjp(_f, q, k, v)
    _grads = _vjp(grad_out)
    _out0 = jnp.asarray(_out)
    return (_out0, *[jnp.asarray(_g) for _g in _grads])
```

```python
import jax, jax.numpy as jnp, math
from jax import lax
import jax.experimental.pallas as pl
import jax.experimental.pallas.tpu as pltpu
NT = (((1,), (1,)), ((), ())); NN = (((1,), (0,)), ((), ())); TN = (((0,), (0,)), ((), ()))
f32 = jnp.float32; bf16 = jnp.bfloat16; u32 = jnp.uint32
T = 128
def dot(a, b, dn=NN): return lax.dot_general(a, b, dn, preferred_element_type=f32)
class Sched:
    def __init__(s, never): s.t = [0] * 4; s.n = 0; s.jobs = []; s.never = never; s.e_end = 0
    def dot(s, a, b, dn=NN):
        x = dot(a, b, dn); m = s.n % 4; s.n += 1
        s.jobs.append((s.t[m], x)); s.t[m] += x.shape[0]; s.last_end = s.t[m]
        return x
    def now(s): return s.t[s.n % 4]
    def pop_at(s, t):
        best = None
        for t0, x in s.jobs:
            i = min(max(-(-(t - t0) // 8), 0), x.shape[0] // 8 - 1); d = abs(t0 + 8 * i - t)
            if best is None or d < best[0]: best = (d, x, i)
        return best[1][best[2] * 8:best[2] * 8 + 8]
def tsum(xs):
    xs = list(xs)
    while len(xs) > 1: xs = [xs[i] + xs[i + 1] if i + 1 < len(xs) else xs[i] for i in range(0, len(xs), 2)]
    return xs[0]
class Buf:
    def __init__(s, ref, z, packed):
        v = lambda i: ref.at[i].bitcast(bf16) if packed else ref.at[i]
        s.wr = v(0); s.rd = v(z); s.half = s.wr.shape[0]; s.dt = bf16 if packed else f32
    def ix(s, a, n):
        h, o = divmod(a, s.half); assert o + n <= s.half
        return slice(o, o + n), slice(h * T, (h + 1) * T)
    def get(s, a, n, fwd=False): return (s.wr if fwd else s.rd)[s.ix(a, n)]
    def put(s, a, x): s.wr[s.ix(a, x.shape[0])] = x.astype(s.dt)
def scratch(Sk):
    big = lambda dt, p: pltpu.VMEM((1, Sk // 2 // p, 2 * T), dt)
    return [big(f32, 1)] * 3 + [big(u32, 2)] * 6 + [pltpu.VMEM((1, T // 2, 2 * T), u32)] * 3 + [big(u32, 2)] * 2
class Head:
    def __init__(s, refs, scr, z, o, sch):
        s.q, s.k, s.v, s.do, s.o, s.dq, s.dk, s.dv = refs
        s.R = o["R"]; s.vt = o["vt"]; s.dqm = o["dqm"]; s.EC = o["EC"]; s.EL = o["EL"]; s.en = o["en"]; s.otie = o["otie"]; s.lpk = o["lpk"]; s.opq = o["opq"]; s.premul = o["premul"]; s.ea = o["ea"]; s.eb = o["eb"]; s.emax = o["emax"]; s.st = {}; s.sch = sch
        zz = lambda n: z if n in s.opq else 0
        s.ss = [Buf(x, zz("s"), False) for x in scr[0:3]]; s.es = [Buf(x, zz("e"), True) for x in scr[3:6]]
        s.dss = [Buf(x, zz("d"), True) for x in scr[6:9]]; s.w = [Buf(x, zz("w"), True) for x in scr[9:12]]
        s.vT = Buf(scr[12], z, True); s.kT = Buf(scr[13], z, True)
        s.Sk = s.k.shape[0]; s.nr = s.Sk // s.R; s.nc = s.Sk // T
        s.scale = s.q.shape[1] ** -0.5; s.c2 = s.scale * math.log2(math.e)
    def rows(s, ref, i, n): return ref[i * n:(i + 1) * n, :]
    def S(s, j, r):
        x = s.sch.dot(s.rows(s.k, r, s.R), s.rows(s.q, j, T), NT)
        if s.premul: x = x * s.c2
        s.ss[j].put(r * s.R, x)
        x = jnp.max(x.reshape(s.R // 8, 8, T), axis=0)
        s.st["m8", j] = x if r == 0 else jnp.maximum(s.st["m8", j], x)
        s.st["send", j] = max(s.sch.last_end, s.st.get(("send", j), 0))
        if r == s.nr - 1: s.st["m", j] = jnp.max(s.st["m8", j], axis=0, keepdims=True)
    def E(s, j, r):
        EC = s.EC
        if r == 0: s.st["mb", j] = jnp.broadcast_to(s.st["m", j], (8, T)); s.st["lh", j] = []
        if r == 0:
            t0 = max(s.st["send", j] + s.ea, s.sch.e_end); t1 = min(s.sch.now() - s.eb, t0 + s.emax)
            s.st["ew", j] = (t0, t1); s.sch.e_end = t1
        for a in range(r * s.R, (r + 1) * s.R, EC):
            lh = s.st["lh", j]; m = s.st["mb", j]
            t0, t1 = s.st["ew", j]; tat = lambda a_: s.sch.pop_at(t0 + (t1 - t0) * a_ // s.Sk)
            if s.en: m = jnp.where(s.sch.never, tat(a), m)
            x = s.ss[j].get(a, EC).reshape(EC // 8, 8, T) - m[None]
            e = jnp.exp2(x if s.premul else x * s.c2)
            s.es[j].put(a, e.reshape(EC, T))
            if s.lpk: e = s.es[j].get(a, EC, True).astype(f32).reshape(EC // 8, 8, T)
            y = tsum([e[i] for i in range(EC // 8)])
            lh.append(jnp.where(s.sch.never, tat(a + s.EL * EC), y if not lh else lh[-1] + y))
        if r == s.nr - 1:
            rr = 1.0 / jnp.sum(lh[-1], axis=0, keepdims=True)
            doT = s.rows(s.do, j, T).T.astype(f32)
            s.st["r", j] = rr
            s.w[j].put(0, doT * rr); s.w[j].put(T, doT * (rr * s.scale))
    def O(s, j, h):
        cs = range(4 * h, 4 * h + 4)
        if s.vt == "lmr": ps = [s.sch.dot(s.rows(s.v, c, T), s.es[j].get(c * T, T), TN) for c in cs]
        else: ps = [s.sch.dot(s.vT.get(c * T, T), s.es[j].get(c * T, T)) for c in cs]
        a = tsum(ps)
        if h == 0: s.st["oacc", j] = a; return
        oT = (s.st["oacc", j] + a) * s.st["r", j]
        s.st["dl", j] = jnp.sum(oT * s.w[j].get(T, T).astype(f32), axis=0, keepdims=True)
        o = oT.T
        s.o[j * T:(j + 1) * T, :] = o.astype(bf16); s.st["otok", j] = o[T - 8:]
    def P(s, j, r):
        dp = s.sch.dot(s.rows(s.v, r, s.R), s.w[j].get(T, T))
        dl = jnp.broadcast_to(s.st["dl", j], (8, T))
        if (j, r) in s.otie: dl = jnp.where(s.sch.never, s.st["otok", s.otie[j, r]], dl)
        x = (dp.reshape(s.R // 8, 8, T) - dl[None]).reshape(s.R, T)
        s.dss[j].put(r * s.R, s.es[j].get(r * s.R, s.R).astype(f32) * x)
    def Q(s, j, h):
        cs = range(4 * h, 4 * h + 4)
        if s.dqm == "lmr": ps = [s.sch.dot(s.dss[j].get(c * T, T), s.rows(s.k, c, T), TN) for c in cs]
        else: ps = [s.sch.dot(s.kT.get(c * T, T), s.dss[j].get(c * T, T)) for c in cs]
        a = tsum(ps)
        if h == 0: s.st["qacc", j] = a; return
        a = (s.st["qacc", j] + a).astype(bf16)
        s.dq[j * T:(j + 1) * T, :] = a if s.dqm == "lmr" else a.T
    def V(s, r):
        s.dv[r * s.R:(r + 1) * s.R, :] = tsum([s.sch.dot(s.es[j].get(r * s.R, s.R), s.w[j].get(0, T), NT) for j in range(3)]).astype(bf16)
    def K(s, r):
        s.dk[r * s.R:(r + 1) * s.R, :] = tsum([s.sch.dot(s.dss[j].get(r * s.R, s.R), s.rows(s.q, j, T)) for j in range(3)]).astype(bf16)
    def X(s, c): s.vT.put(c * T, s.rows(s.v, c, T).T)
    def Y(s, c): s.kT.put(c * T, s.rows(s.k, c, T).T)
    def run(s, t):
        dict(S=s.S, E=s.E, O=s.O, P=s.P, Q=s.Q, V=s.V, K=s.K, X=s.X, Y=s.Y)[t[0]](*t[1:])
    def expand(s, w):
        n = w[0]; a = [int(x) for x in w[1:]]
        if n in "SEP": return [(n, a[0], r) for r in (range(s.nr) if len(a) == 1 else a[1:])]
        if n in "OQ": return [(n, a[0], h) for h in (range(2) if len(a) == 1 else a[1:])]
        if n in "XY": return [(n, c) for c in (range(s.nc) if not a else a)]
        return [(n, r) for r in (range(s.nr) if not a else a)]
ORDER = "S0 S1 -K0 S20 -K1 S21 -K2 S22 -K3 S23 E0 O0 E1 O1 P0 E2 O2 P1 Q0 V0 P20 V1 P21 V2 P22 V3 P23 Q1 Q2"
FIRST = ORDER.replace("E0 O0", "+S0 E0 O0")
def make(G=1, U=1, order=ORDER, first=FIRST, NB=2, **kw):
    o = dict(R=256, vt="lmr", dqm="lmr", EC=64, EL=1, en=True, otie={(1, 0): 0, (2, 0): 1, (2, 2): 2}, lpk=False, opq="sedw", premul=False, ea=32, eb=200, emax=500); o.update(kw)
    if o["vt"] != "lmr" and "X" not in order: order = "X " + order
    if o["dqm"] != "lmr" and "Y" not in order: order = order.replace("P0", "Y P0")
    def group(refs_list, scr, z):
        n = len(scr) // NB
        sch = Sched(jnp.broadcast_to(z, (8, T)) > 0)
        hs = [Head(r, scr[(u % NB) * n:(u % NB + 1) * n], z, o, sch) for u, r in enumerate(refs_list)]
        done = set()
        for u in range(len(hs) + 1):
            for w in (first if u == 0 and first else order).split():
                hi = u + {"-": -1, "+": 1}.get(w[0], 0)
                if 0 <= hi < len(hs):
                    for t in hs[hi].expand(w.lstrip("-+")):
                        if (hi, t) not in done: done.add((hi, t)); hs[hi].run(t)
    def kern(*refs):
        refs, scr = refs[:8], refs[8:]
        z = lax.shift_right_logical(pl.program_id(0), 24)
        def body(i, _): group([[r.at[i * U + u] for r in refs] for u in range(U)], scr, z)
        if G == U: body(0, None)
        else: lax.fori_loop(0, G // U, body, None)
    @jax.jit
    def fn(q, k, v, do):
        B, H, Sq, D = q.shape; Sk = k.shape[2]; N = B * H
        r = lambda x: x.reshape(N, x.shape[2], D)
        sq = pl.BlockSpec((G, Sq, D), lambda i: (i, 0, 0)); sk = pl.BlockSpec((G, Sk, D), lambda i: (i, 0, 0))
        oq = jax.ShapeDtypeStruct((N, Sq, D), q.dtype); ok = jax.ShapeDtypeStruct((N, Sk, D), q.dtype)
        outs = pl.pallas_call(kern, grid=(N // G,), in_specs=[sq, sk, sk, sq], out_specs=[sq, sq, sk, sk],
            out_shape=[oq, oq, ok, ok], scratch_shapes=scratch(Sk) * NB,
            compiler_params=pltpu.CompilerParams(dimension_semantics=("parallel",), vmem_limit_bytes=100 * 2**20))(r(q), r(k), r(v), r(do))
        return tuple(x.reshape(B, H, x.shape[1], D) for x in outs)
    return fn

_impl = make(G=4, U=4)
@jax.jit
def pallas_standalone__mha_softmax__near_ridge_kernel(q, k, v, grad_out):
    return _impl(q, k, v, grad_out)
```

```python
import jax, jax.numpy as jnp, math
from jax import lax
import jax.experimental.pallas as pl
import jax.experimental.pallas.tpu as pltpu
NT = (((1,), (1,)), ((), ())); NN = (((1,), (0,)), ((), ())); TN = (((0,), (0,)), ((), ()))
f32 = jnp.float32; bf16 = jnp.bfloat16; u32 = jnp.uint32
T = 128
def dot(a, b, dn=NN): return lax.dot_general(a, b, dn, preferred_element_type=f32)
class Sched:
    def __init__(s, never): s.t = [0] * 4; s.n = 0; s.jobs = []; s.never = never; s.e_end = 0
    def dot(s, a, b, dn=NN):
        x = dot(a, b, dn); m = s.n % 4; s.n += 1
        s.jobs.append((s.t[m], x)); s.t[m] += x.shape[0]; s.last_end = s.t[m]
        return x
    def now(s): return s.t[s.n % 4]
    def pop_at(s, t):
        best = None
        for t0, x in s.jobs:
            i = min(max(-(-(t - t0) // 8), 0), x.shape[0] // 8 - 1); d = abs(t0 + 8 * i - t)
            if best is None or d < best[0]: best = (d, x, i)
        return best[1][best[2] * 8:best[2] * 8 + 8]
def tsum(xs):
    xs = list(xs)
    while len(xs) > 1: xs = [xs[i] + xs[i + 1] if i + 1 < len(xs) else xs[i] for i in range(0, len(xs), 2)]
    return xs[0]
class Buf:
    def __init__(s, ref, z, packed):
        v = lambda i: ref.at[i].bitcast(bf16) if packed else ref.at[i]
        s.wr = v(0); s.rd = v(z); s.half = s.wr.shape[0]; s.dt = bf16 if packed else f32
    def ix(s, a, n):
        h, o = divmod(a, s.half); assert o + n <= s.half
        return slice(o, o + n), slice(h * T, (h + 1) * T)
    def get(s, a, n, fwd=False): return (s.wr if fwd else s.rd)[s.ix(a, n)]
    def put(s, a, x): s.wr[s.ix(a, x.shape[0])] = x.astype(s.dt)
def scratch(Sk):
    big = lambda dt, p: pltpu.VMEM((1, Sk // 2 // p, 2 * T), dt)
    return [big(f32, 1)] * 3 + [big(u32, 2)] * 6 + [pltpu.VMEM((1, T // 2, 2 * T), u32)] * 3 + [big(u32, 2)] * 2
class Head:
    def __init__(s, refs, scr, z, o, sch):
        s.q, s.k, s.v, s.do, s.o, s.dq, s.dk, s.dv = refs
        s.R = o["R"]; s.vt = o["vt"]; s.dqm = o["dqm"]; s.EC = o["EC"]; s.EL = o["EL"]; s.en = o["en"]; s.WC = o["WC"]; s.wd = o["wd"]; s.ws = o["ws"]; s.ib = o["ib"]; s.otie = o["otie"]; s.lpk = o["lpk"]; s.opq = o["opq"]; s.premul = o["premul"]; s.ea = o["ea"]; s.eb = o["eb"]; s.emax = o["emax"]; s.st = {}; s.sch = sch
        zz = lambda n: z if n in s.opq else 0
        s.ss = [Buf(x, zz("s"), False) for x in scr[0:3]]; s.es = [Buf(x, zz("e"), True) for x in scr[3:6]]
        s.dss = [Buf(x, zz("d"), True) for x in scr[6:9]]; s.w = [Buf(x, zz("w"), True) for x in scr[9:12]]
        s.vT = Buf(scr[12], z, True); s.kT = Buf(scr[13], z, True)
        s.Sk = s.k.shape[0]; s.nr = s.Sk // s.R; s.nc = s.Sk // T
        s.scale = s.q.shape[1] ** -0.5; s.c2 = s.scale * math.log2(math.e)
    def rows(s, ref, i, n):
        if s.ib: return pltpu.bitcast(ref.bitcast(u32)[i * n // 2:(i + 1) * n // 2, :], bf16)
        return ref[i * n:(i + 1) * n, :]
    def S(s, j, r):
        x = s.sch.dot(s.rows(s.k, r, s.R), s.rows(s.q, j, T), NT)
        if s.premul: x = x * s.c2
        s.ss[j].put(r * s.R, x)
        x = jnp.max(x.reshape(s.R // 8, 8, T), axis=0)
        s.st["m8", j] = x if r == 0 else jnp.maximum(s.st["m8", j], x)
        s.st["send", j] = max(s.sch.last_end, s.st.get(("send", j), 0))
        if r == s.nr - 1: s.st["m", j] = jnp.max(s.st["m8", j], axis=0, keepdims=True)
    def E(s, j, r):
        EC = s.EC
        if r == 0: s.st["mb", j] = jnp.broadcast_to(s.st["m", j], (8, T)); s.st["lh", j] = []
        if r == 0:
            t0 = max(s.st["send", j] + s.ea, s.sch.e_end); t1 = min(s.sch.now() - s.eb, t0 + s.emax)
            s.st["ew", j] = (t0, t1); s.sch.e_end = t1
        for a in range(r * s.R, (r + 1) * s.R, EC):
            lh = s.st["lh", j]; m = s.st["mb", j]
            t0, t1 = s.st["ew", j]; tat = lambda a_: s.sch.pop_at(t0 + (t1 - t0) * a_ // s.Sk)
            if s.en: m = jnp.where(s.sch.never, tat(a), m)
            x = s.ss[j].get(a, EC).reshape(EC // 8, 8, T) - m[None]
            e = jnp.exp2(x if s.premul else x * s.c2)
            s.es[j].put(a, e.reshape(EC, T))
            if s.lpk: e = s.es[j].get(a, EC, True).astype(f32).reshape(EC // 8, 8, T)
            y = tsum([e[i] for i in range(EC // 8)])
            lh.append(jnp.where(s.sch.never, tat(a + s.EL * EC), y if not lh else lh[-1] + y))
    def W(s, j):
        rr = 1.0 / jnp.sum(s.st["lh", j][-1], axis=0, keepdims=True)
        s.st["r", j] = rr; r8 = jnp.broadcast_to(rr, (8, T))
        doT = s.rows(s.do, j, T).T.astype(f32); WC = s.WC
        t = s.st["ew", j][1] + s.wd
        for c in range(T // WC):
            rc = jnp.where(s.sch.never, s.sch.pop_at(t + c * s.ws), r8) if s.ws else r8
            x = doT[c * WC:(c + 1) * WC].reshape(WC // 8, 8, T)
            s.w[j].put(c * WC, (x * rc[None]).reshape(WC, T)); s.w[j].put(T + c * WC, (x * (rc * s.scale)[None]).reshape(WC, T))
    def O(s, j, h):
        cs = range(4 * h, 4 * h + 4)
        if s.vt == "lmr": ps = [s.sch.dot(s.rows(s.v, c, T), s.es[j].get(c * T, T), TN) for c in cs]
        else: ps = [s.sch.dot(s.vT.get(c * T, T), s.es[j].get(c * T, T)) for c in cs]
        a = tsum(ps)
        if h == 0: s.st["oacc", j] = a; return
        s.W(j)
        oT = (s.st["oacc", j] + a) * s.st["r", j]
        s.st["dl", j] = jnp.sum(oT * s.w[j].get(T, T).astype(f32), axis=0, keepdims=True)
        o = oT.T
        s.o[j * T:(j + 1) * T, :] = o.astype(bf16); s.st["otok", j] = o[T - 8:]
    def P(s, j, r):
        dp = s.sch.dot(s.rows(s.v, r, s.R), s.w[j].get(T, T))
        dl = jnp.broadcast_to(s.st["dl", j], (8, T))
        if (j, r) in s.otie: dl = jnp.where(s.sch.never, s.st["otok", s.otie[j, r]], dl)
        x = (dp.reshape(s.R // 8, 8, T) - dl[None]).reshape(s.R, T)
        s.dss[j].put(r * s.R, s.es[j].get(r * s.R, s.R).astype(f32) * x)
    def Q(s, j, h):
        cs = range(4 * h, 4 * h + 4)
        if s.dqm == "lmr": ps = [s.sch.dot(s.dss[j].get(c * T, T), s.rows(s.k, c, T), TN) for c in cs]
        else: ps = [s.sch.dot(s.kT.get(c * T, T), s.dss[j].get(c * T, T)) for c in cs]
        a = tsum(ps)
        if h == 0: s.st["qacc", j] = a; return
        a = (s.st["qacc", j] + a).astype(bf16)
        s.dq[j * T:(j + 1) * T, :] = a if s.dqm == "lmr" else a.T
    def V(s, r):
        s.dv[r * s.R:(r + 1) * s.R, :] = tsum([s.sch.dot(s.es[j].get(r * s.R, s.R), s.w[j].get(0, T), NT) for j in range(3)]).astype(bf16)
    def K(s, r):
        s.dk[r * s.R:(r + 1) * s.R, :] = tsum([s.sch.dot(s.dss[j].get(r * s.R, s.R), s.rows(s.q, j, T)) for j in range(3)]).astype(bf16)
    def X(s, c): s.vT.put(c * T, s.rows(s.v, c, T).T)
    def Y(s, c): s.kT.put(c * T, s.rows(s.k, c, T).T)
    def run(s, t):
        dict(S=s.S, E=s.E, O=s.O, P=s.P, Q=s.Q, V=s.V, K=s.K, X=s.X, Y=s.Y)[t[0]](*t[1:])
    def expand(s, w):
        n = w[0]; a = [int(x) for x in w[1:]]
        if n in "SEP": return [(n, a[0], r) for r in (range(s.nr) if len(a) == 1 else a[1:])]
        if n in "OQ": return [(n, a[0], h) for h in (range(2) if len(a) == 1 else a[1:])]
        if n in "XY": return [(n, c) for c in (range(s.nc) if not a else a)]
        return [(n, r) for r in (range(s.nr) if not a else a)]
ORDER = "S0 S1 -K0 S20 -K1 S21 -K2 S22 -K3 S23 E0 O0 E1 O1 P0 E2 O2 P1 Q0 V0 P20 V1 P21 V2 P22 V3 P23 Q1 Q2"
FIRST = ORDER.replace("E0 O0", "+S0 E0 O0")
def make(G=1, U=1, order=ORDER, first=FIRST, NB=2, **kw):
    o = dict(R=256, vt="lmr", dqm="lmr", EC=64, EL=1, en=True, WC=16, wd=64, ws=16, ib=True, otie={(1, 0): 0, (2, 0): 1, (2, 2): 2}, lpk=False, opq="sedw", premul=False, ea=32, eb=260, emax=500); o.update(kw)
    if o["vt"] != "lmr" and "X" not in order: order = order.replace("E0 O0", "X E0 O0"); first = first.replace("E0 O0", "X E0 O0")
    if o["dqm"] != "lmr" and "Y" not in order: order = order.replace("P0", "Y P0")
    def group(refs_list, scr, z):
        n = len(scr) // NB
        sch = Sched(jnp.broadcast_to(z, (8, T)) > 0)
        hs = [Head(r, scr[(u % NB) * n:(u % NB + 1) * n], z, o, sch) for u, r in enumerate(refs_list)]
        done = set()
        for u in range(len(hs) + 1):
            for w in (first if u == 0 and first else order).split():
                hi = u + {"-": -1, "+": 1}.get(w[0], 0)
                if 0 <= hi < len(hs):
                    for t in hs[hi].expand(w.lstrip("-+")):
                        if (hi, t) not in done: done.add((hi, t)); hs[hi].run(t)
    def kern(*refs):
        refs, scr = refs[:8], refs[8:]
        z = lax.shift_right_logical(pl.program_id(0), 24)
        def body(i, _): group([[r.at[i * U + u] for r in refs] for u in range(U)], scr, z)
        if G == U: body(0, None)
        else: lax.fori_loop(0, G // U, body, None)
    @jax.jit
    def fn(q, k, v, do):
        B, H, Sq, D = q.shape; Sk = k.shape[2]; N = B * H
        r = lambda x: x.reshape(N, x.shape[2], D)
        sq = pl.BlockSpec((G, Sq, D), lambda i: (i, 0, 0)); sk = pl.BlockSpec((G, Sk, D), lambda i: (i, 0, 0))
        oq = jax.ShapeDtypeStruct((N, Sq, D), q.dtype); ok = jax.ShapeDtypeStruct((N, Sk, D), q.dtype)
        outs = pl.pallas_call(kern, grid=(N // G,), in_specs=[sq, sk, sk, sq], out_specs=[sq, sq, sk, sk],
            out_shape=[oq, oq, ok, ok], scratch_shapes=scratch(Sk) * NB,
            compiler_params=pltpu.CompilerParams(dimension_semantics=("parallel",), vmem_limit_bytes=100 * 2**20))(r(q), r(k), r(v), r(do))
        return tuple(x.reshape(B, H, x.shape[1], D) for x in outs)
    return fn

_impl = make(G=8, U=8)
@jax.jit
def pallas_standalone__mha_softmax__near_ridge_kernel(q, k, v, grad_out):
    return _impl(q, k, v, grad_out)
```

```python
import math
import jax
import jax.numpy as jnp
from jax import lax
import jax.experimental.pallas as pl
import jax.experimental.pallas.tpu as pltpu
NT = (((1,), (1,)), ((), ())); NN = (((1,), (0,)), ((), ())); TN = (((0,), (0,)), ((), ()))
f32 = jnp.float32; bf16 = jnp.bfloat16; u32 = jnp.uint32
T = 128
R = 256
U, A = 9, 4
EC, WC = 16, 16
EA, EB, EMAX, WD, WS = 32, 300, 500, 64, 16
OTIE = {(1, 0): 0, (2, 0): 1, (2, 2): 2}


def dot(a, b, dn=NN): return lax.dot_general(a, b, dn, preferred_element_type=f32)


class Sched:
    def __init__(s, never): s.t = [0] * 4; s.n = 0; s.jobs = []; s.never = never; s.e_end = 0
    def dot(s, a, b, dn=NN):
        x = dot(a, b, dn); m = s.n % 4; s.n += 1
        s.jobs.append((s.t[m], x)); s.t[m] += x.shape[0]; s.last_end = s.t[m]
        return x
    def now(s): return s.t[s.n % 4]
    def pop_at(s, t):
        best = None
        for t0, x in s.jobs:
            i = min(max(-(-(t - t0) // 8), 0), x.shape[0] // 8 - 1); d = abs(t0 + 8 * i - t)
            if best is None or d < best[0]: best = (d, x, i)
        return best[1][best[2] * 8:best[2] * 8 + 8]


def tsum(xs):
    xs = list(xs)
    while len(xs) > 1: xs = [xs[i] + xs[i + 1] if i + 1 < len(xs) else xs[i] for i in range(0, len(xs), 2)]
    return xs[0]


class Buf:
    def __init__(s, ref, z, packed):
        v = lambda i: ref.at[i].bitcast(bf16) if packed else ref.at[i]
        s.wr = v(0); s.rd = v(z); s.half = s.wr.shape[0]; s.dt = bf16 if packed else f32
    def ix(s, a, n):
        h, o = divmod(a, s.half); assert o + n <= s.half
        return slice(o, o + n), slice(h * T, (h + 1) * T)
    def get(s, a, n): return s.rd[s.ix(a, n)]
    def put(s, a, x): s.wr[s.ix(a, x.shape[0])] = x.astype(s.dt)


def scratch(Sk):
    big = lambda dt, p: pltpu.VMEM((1, Sk // 2 // p, 2 * T), dt)
    return [big(f32, 1)] * 3 + [big(u32, 2)] * 6 + [pltpu.VMEM((1, T // 2, 2 * T), u32)] * 3


class Head:
    def __init__(s, refs, scr, z, sch):
        s.q, s.k, s.v, s.do, s.o, s.dq, s.dk, s.dv = refs
        s.st = {}; s.sch = sch
        s.ss = [Buf(x, z, False) for x in scr[0:3]]; s.es = [Buf(x, z, True) for x in scr[3:6]]
        s.dss = [Buf(x, z, True) for x in scr[6:9]]; s.w = [Buf(x, z, True) for x in scr[9:12]]
        s.Sk = s.k.shape[0]; s.nr = s.Sk // R; s.nc = s.Sk // T
        s.scale = s.q.shape[1] ** -0.5; s.c2 = s.scale * math.log2(math.e)
    def rows(s, ref, i, n):
        return pltpu.bitcast(ref.bitcast(u32)[i * n // 2:(i + 1) * n // 2, :], bf16)
    def S(s, j, r):
        x = s.sch.dot(s.rows(s.k, r, R), s.rows(s.q, j, T), NT)
        s.ss[j].put(r * R, x)
        x = jnp.max(x.reshape(R // 8, 8, T), axis=0)
        s.st["m8", j] = x if r == 0 else jnp.maximum(s.st["m8", j], x)
        s.st["send", j] = max(s.sch.last_end, s.st.get(("send", j), 0))
        if r == s.nr - 1: s.st["m", j] = jnp.max(s.st["m8", j], axis=0, keepdims=True)
    def E(s, j, r):
        if r == 0: s.st["mb", j] = jnp.broadcast_to(s.st["m", j], (8, T)); s.st["lh", j] = []
        if r == 0:
            t0 = max(s.st["send", j] + EA, s.sch.e_end); t1 = min(s.sch.now() - EB, t0 + EMAX)
            s.st["ew", j] = (t0, t1); s.sch.e_end = t1
        for a in range(r * R, (r + 1) * R, EC):
            lh = s.st["lh", j]; m = s.st["mb", j]
            t0, t1 = s.st["ew", j]; tat = lambda a_: s.sch.pop_at(t0 + (t1 - t0) * a_ // s.Sk)
            m = lax.select(s.sch.never, tat(a), m)
            x = s.ss[j].get(a, EC).reshape(EC // 8, 8, T) - m[None]
            e = jnp.exp2(x * s.c2)
            s.es[j].put(a, e.reshape(EC, T))
            y = tsum([e[i] for i in range(EC // 8)])
            lh.append(lax.select(s.sch.never, tat(a + EC), y if not lh else lh[-1] + y))
    def W(s, j):
        rr = 1.0 / jnp.sum(s.st["lh", j][-1], axis=0, keepdims=True)
        s.st["r", j] = rr; r8 = jnp.broadcast_to(rr, (8, T))
        doT = s.rows(s.do, j, T).T.astype(f32)
        t = s.st["ew", j][1] + WD
        for c in range(T // WC):
            rc = lax.select(s.sch.never, s.sch.pop_at(t + c * WS), r8)
            x = doT[c * WC:(c + 1) * WC].reshape(WC // 8, 8, T)
            s.w[j].put(c * WC, (x * rc[None]).reshape(WC, T)); s.w[j].put(T + c * WC, (x * (rc * s.scale)[None]).reshape(WC, T))
    def O(s, j, h):
        cs = range(4 * h, 4 * h + 4)
        ps = [s.sch.dot(s.rows(s.v, c, T), s.es[j].get(c * T, T), TN) for c in cs]
        a = tsum(ps)
        if h == 0: s.st["oacc", j] = a; return
        s.W(j)
        oT = (s.st["oacc", j] + a) * s.st["r", j]
        s.st["dl", j] = jnp.sum(oT * s.w[j].get(T, T).astype(f32), axis=0, keepdims=True)
        o = oT.T
        s.o[j * T:(j + 1) * T, :] = o.astype(bf16); s.st["otok", j] = o[T - 8:]
    def P(s, j, r):
        dp = s.sch.dot(s.rows(s.v, r, R), s.w[j].get(T, T))
        dl = jnp.broadcast_to(s.st["dl", j], (8, T))
        if (j, r) in OTIE: dl = lax.select(s.sch.never, s.st["otok", OTIE[j, r]], dl)
        x = (dp.reshape(R // 8, 8, T) - dl[None]).reshape(R, T)
        s.dss[j].put(r * R, s.es[j].get(r * R, R).astype(f32) * x)
    def Q(s, j, h):
        cs = range(4 * h, 4 * h + 4)
        ps = [s.sch.dot(s.dss[j].get(c * T, T), s.rows(s.k, c, T), TN) for c in cs]
        a = tsum(ps)
        if h == 0: s.st["qacc", j] = a; return
        a = (s.st["qacc", j] + a).astype(bf16)
        s.dq[j * T:(j + 1) * T, :] = a
    def V(s, r):
        s.dv[r * R:(r + 1) * R, :] = tsum([s.sch.dot(s.es[j].get(r * R, R), s.w[j].get(0, T), NT) for j in range(3)]).astype(bf16)
    def K(s, r):
        s.dk[r * R:(r + 1) * R, :] = tsum([s.sch.dot(s.dss[j].get(r * R, R), s.rows(s.q, j, T)) for j in range(3)]).astype(bf16)
    def run(s, t): dict(S=s.S, E=s.E, O=s.O, P=s.P, Q=s.Q, V=s.V, K=s.K)[t[0]](*t[1:])
    def expand(s, w):
        n = w[0]; a = [int(x) for x in w[1:]]
        if n in "SEP": return [(n, a[0], r) for r in (range(s.nr) if len(a) == 1 else a[1:])]
        if n in "OQ": return [(n, a[0], h) for h in (range(2) if len(a) == 1 else a[1:])]
        return [(n, r) for r in (range(s.nr) if not a else a)]


ORDER = "S0 S1 -K0 S20 -K1 S21 -K2 S22 -K3 S23 E0 O0 E1 O1 P0 E2 O2 P1 P20 V0 P21 V1 Q0 P22 V2 P23 V3 Q1 Q2"
FIRST = ORDER.replace("E0 O0", "+S0 E0 O0").replace("S1", "D S1")


def group(refs_list, scr, z, hook):
    n = len(scr) // 2
    sch = Sched(jnp.broadcast_to(z, (8, T)) > 0)
    hs = [Head(r, scr[(u % 2) * n:(u % 2 + 1) * n], z, sch) for u, r in enumerate(refs_list)]
    done = set()
    for u in range(len(hs) + 1):
        for w in (FIRST if u == 0 else ORDER).split():
            if w == "D":
                hook()
                continue
            hi = u + {"-": -1, "+": 1}.get(w[0], 0)
            if 0 <= hi < len(hs):
                for t in hs[hi].expand(w.lstrip("-+")):
                    if (hi, t) not in done: done.add((hi, t)); hs[hi].run(t)


def kern(*refs):
    hin, hout, bin_, bout = refs[0:4], refs[4:8], refs[8:12], refs[12:16]
    sbi, sbo, ssi, sso = refs[16:20]; scr = refs[20:]
    N = hin[0].shape[0]; M = (N - 2 * A) // U; ls = M & 1
    opaque = lambda i: lax.shift_right_logical(i, 24)
    big_in = lambda h0, s_: [pltpu.make_async_copy(hin[t].at[pl.ds(h0, U)], bin_[t].at[s_], sbi.at[s_, t]) for t in range(4)]
    big_out = lambda h0, s_: [pltpu.make_async_copy(bout[t].at[s_], hout[t].at[pl.ds(h0, U)], sbo.at[s_, t]) for t in range(4)]
    one_in = lambda h: [pltpu.make_async_copy(hin[t].at[h], bin_[t].at[0, h], ssi.at[h, t]) for t in range(4)]
    one_out = lambda g: [pltpu.make_async_copy(bout[t].at[2, U - A + g], hout[t].at[N - A + g], sso.at[g, t]) for t in range(4)]
    lead_out = lambda: [pltpu.make_async_copy(bout[t].at[2, pl.ds(0, A)], hout[t].at[pl.ds(0, A)], sbo.at[2, t]) for t in range(4)]
    def start(cs):
        for c in cs: c.start()
    def wait(cs):
        for c in cs: c.wait()
    def main(i, c):
        slot = i & 1; h0 = i * U - (U - A)
        wait(big_in(h0, slot))
        pl.when(i > 2)(lambda: wait(big_out(h0 - 2 * U, slot)))
        def hook():
            pl.when(i > 1)(lambda: start(big_out(h0 - U, 1 - slot)))
            start(big_in(jnp.minimum(h0 + U, N - U), 1 - slot))
        group([[r.at[slot, u] for r in bin_ + bout] for u in range(U)], scr, opaque(i), hook)
        return c
    def phase(p, c):
        def ramp(g, c):
            pl.when(p == 0)(lambda: wait(one_in(g)))
            def hook():
                pl.when((p == 0) & (g == 0))(lambda: start(sum([one_in(a) for a in range(1, A)], [])))
                pl.when((p == 0) & (g == 1))(lambda: start(big_in(A, 1)))
            h = g + p * (U - A)
            group([[r.at[p * (1 - ls), h] for r in bin_] + [r.at[2, h] for r in bout]], scr, opaque(g), hook)
            pl.when(p == 1)(lambda: start(one_out(g)))
            return c
        lax.fori_loop(0, A, ramp, 0)
        @pl.when(p == 0)
        def _():
            start(lead_out())
            lax.fori_loop(1, M + 1, main, 0)
            start(big_out(N - U - A, ls))
            wait(big_in(N - U, 1 - ls))
            wait(lead_out())
        return c
    start(one_in(0))
    lax.fori_loop(0, 2, phase, 0)
    wait(big_out(N - 2 * U - A, 1 - ls)); wait(big_out(N - U - A, ls))
    for g in range(A): wait(one_out(g))


@jax.jit
def pallas_standalone__mha_softmax__near_ridge_kernel(q, k, v, grad_out):
    B, H, Sq, D = q.shape; Sk = k.shape[2]; N = B * H
    assert (N - 2 * A) % U == 0 and N - 2 * A >= 2 * U and (Sq, Sk, D) == (3 * T, 4 * R, T)
    r = lambda x: x.reshape(N, x.shape[2], D)
    hbm = pl.BlockSpec(memory_space=pl.ANY)
    oq = jax.ShapeDtypeStruct((N, Sq, D), q.dtype); ok = jax.ShapeDtypeStruct((N, Sk, D), q.dtype)
    buf = lambda n, S: pltpu.VMEM((n, U, S, D), q.dtype)
    sem = pltpu.SemaphoreType.DMA
    outs = pl.pallas_call(kern, in_specs=[hbm] * 4, out_specs=[hbm] * 4, out_shape=[oq, oq, ok, ok],
        scratch_shapes=[buf(2, S) for S in (Sq, Sk, Sk, Sq)] + [buf(3, S) for S in (Sq, Sq, Sk, Sk)] + [sem((2, 4)), sem((3, 4)), sem((A, 4)), sem((A, 4))] + scratch(Sk) * 2,
        compiler_params=pltpu.CompilerParams(vmem_limit_bytes=100 * 2**20, disable_bounds_checks=True))(r(q), r(k), r(v), r(grad_out))
    return tuple(x.reshape(B, H, x.shape[1], D) for x in outs)
```
